```python
import os as _os
_os.environ.setdefault("JAX_PLATFORMS", "cpu")
import jax
import jax.numpy as jnp

def _softmax(x, axis=-1):
    return jax.nn.softmax(x, axis=axis)
def _gelu(x):
    return jax.nn.gelu(x, approximate=True)
def _silu(x):
    return jax.nn.silu(x)
def _sigmoid(x):
    return jax.nn.sigmoid(x)
def _layernorm(x, axis=-1, eps=1e-5):
    m = jnp.mean(x, axis=axis, keepdims=True)
    v = jnp.var(x, axis=axis, keepdims=True)
    return (x - m) / jnp.sqrt(v + eps)
def _scatter_add(tgt, idx, src, axis=0):
    return tgt.at[idx].add(src)
def _segment_sum(src, seg, n):
    return jax.ops.segment_sum(src, seg, n)
class _Rng:
    def __init__(self, key):
        self._k = key
    def _next(self):
        self._k, sub = jax.random.split(self._k)
        return sub
    def normal(self, shape):
        return jax.random.normal(self._next(), shape, dtype=jnp.bfloat16)
    def randint(self, lo, hi, shape):
        return jax.random.randint(self._next(), shape, lo, hi, dtype=jnp.int32)
    def uniform(self, shape, lo=0.0, hi=1.0):
        return jax.random.uniform(self._next(), shape, jnp.bfloat16, lo, hi)
    def permutation(self, n):
        return jax.random.permutation(self._next(), n)


kernel_name = 'sequential_preLN__mha_block__mixer_token_mlp__prompt'

def setup_inputs():
    _rng = _Rng(jax.random.key(int.from_bytes(__import__("os").urandom(4), "little")))
    _w = (lambda a: (lambda t: t.astype(jnp.bfloat16) if jnp.issubdtype(t.dtype, jnp.floating) else t)(jnp.asarray(a)))
    def _A_setup():
        B, S, D, H = 1, 2048, 448, 16
        return {
            "x": _w((lambda *s: _rng.normal(s) * 0.05)(B, S, D)),
            "wqkv": _w((lambda *s: _rng.normal(s) * 0.05)(D, 3 * D)),
            "wo": _w((lambda *s: _rng.normal(s) * 0.05)(D, D)),
        }
    _A_in = _A_setup()

    def _B_setup():
        B, S, D, F = 1, 2048, 448, 1792
        return {
            "x": _w((lambda *s: _rng.normal(s) * 0.05)(B, S, D)),
            "w1": _w((lambda *s: _rng.normal(s) * 0.2)(S, F) * (S ** -0.5)),
            "b1": _w((lambda *s: _rng.normal(s) * 0.2)(F) * 0.02),
            "w2": _w((lambda *s: _rng.normal(s) * 0.2)(F, S) * (F ** -0.5)),
            "b2": _w((lambda *s: _rng.normal(s) * 0.05)(S) * 0.02),
        }
    _B_in = _B_setup()

    return {
        "A_x": _A_in["x"],
        "A_wqkv": _A_in["wqkv"],
        "A_wo": _A_in["wo"],
        "B_x": _B_in["x"],
        "B_w1": _B_in["w1"],
        "B_b1": _B_in["b1"],
        "B_w2": _B_in["w2"],
        "B_b2": _B_in["b2"],
    }

def reference(A_x, A_wqkv, A_wo, B_x, B_w1, B_b1, B_w2, B_b2):
    def _A_ref(x, wqkv, wo):
        B, S, D = x.shape
        H = 16
        Dh = D // H
        qkv = (lambda x, *d: x.transpose(*d))((x @ wqkv).reshape(B, S, 3, H, Dh), 2, 0, 3, 1, 4)
        q, k, v = qkv[0], qkv[1], qkv[2]
        scores = jnp.einsum("bhqd,bhkd->bhqk", q, k) * (Dh ** -0.5)
        p = _softmax(scores, axis=-1)
        o = jnp.einsum("bhqk,bhkd->bhqd", p, v)
        return (lambda x, *d: x.transpose(*d))(o, 0, 2, 1, 3).reshape(B, S, D) @ wo

    def _B_ref(x, w1, b1, w2, b2):
        B, S, D = x.shape
        h = _layernorm(x, axis=-1)
        u = jnp.einsum("bsd,sf->bdf", h, w1) + b1
        u = _gelu(u)
        y = jnp.einsum("bdf,fs->bds", u, w2) + b2
        return (lambda x, *d: x.transpose(*d))(y, 0, 2, 1)

    x = A_x
    h = x + _A_ref(_layernorm(x, axis=-1), A_wqkv, A_wo)
    h2 = h + _B_ref(_layernorm(h, axis=-1), B_w1, B_b1, B_w2, B_b2)
    return h2
```

```python
import functools
import math

import jax
import jax.numpy as jnp
import jax.experimental.pallas as pl
import jax.experimental.pallas.tpu as pltpu

S = 2048
D = 448
H = 16
DH = 28
F = 1792
GW = 112
HP = 32
DP = H * HP
EPS = 1e-5
QSCALE = (DH ** -0.5) * math.log2(math.e)

TQ = 512
NH = 2
TB = TQ * NH
NQ = S // TB
LQ = NQ.bit_length() - 1
TK = 128
NC = S // TK
NBLK = H * NQ

F32 = jnp.float32
BF16 = jnp.bfloat16


def _nt_dot(a, b):
    return jax.lax.dot_general(a, b, (((1,), (1,)), ((), ())),
                               preferred_element_type=F32)


def _dot(a, b):
    return jnp.dot(a, b, preferred_element_type=F32)


def _kernel(x_hbm, wqkv_hbm, wo_hbm, w1_hbm, w2_hbm, b1_ref, b2_ref,
            o_hbm,
            x_v, wqkv_v, wo_v, w1_v, w2_v,
            wqvT_v, wk_v, woT_v,
            xn_v, xT_v, k_v, qT_v, vT_v, oT_v,
            sA, sB, m_ref, hT_v, hnT_v, g_v, out_v,
            sems):
    cp_wqkv = pltpu.make_async_copy(wqkv_hbm, wqkv_v, sems.at[0])
    cp_x = pltpu.make_async_copy(x_hbm, x_v, sems.at[1])
    cp_wo = pltpu.make_async_copy(wo_hbm, wo_v, sems.at[2])
    cp_w1 = pltpu.make_async_copy(w1_hbm, w1_v, sems.at[3])
    cp_w2 = pltpu.make_async_copy(w2_hbm, w2_v, sems.at[4])
    cp_wqkv.start()
    cp_x.start()
    cp_wo.start()
    cp_w1.start()
    cp_w2.start()

    cp_wqkv.wait()
    wqvT_v[0:D, :] = wqkv_v[:, 0:D].T
    wqvT_v[D:D + DP, :] = jnp.zeros((DP, D), BF16)
    wvT = wqkv_v[:, 2 * D:3 * D].astype(F32).T
    for h in range(H):
        wqvT_v[D + HP * h:D + HP * h + DH, :] = wvT[DH * h:DH * h + DH, :].astype(BF16)
    wk_v[...] = jnp.zeros((D, DP), BF16)
    for g in range(4):
        wk_v[:, 128 * g:128 * g + GW] = wqkv_v[:, D + GW * g:D + GW * g + GW]

    cp_x.wait()
    xf = x_v[...].astype(F32)
    mu = jnp.mean(xf, axis=-1, keepdims=True)
    xc = xf - mu
    var = jnp.mean(xc * xc, axis=-1, keepdims=True)
    xn_v[...] = (xc * jax.lax.rsqrt(var + EPS)).astype(BF16)
    xT_v[...] = xf.T

    k_v[...] = _dot(xn_v[...], wk_v[...]).astype(BF16)
    qT_v[0:D, :] = (_nt_dot(wqvT_v[0:D, :], xn_v[...]) * QSCALE).astype(BF16)
    qT_v[D:DP, :] = jnp.zeros((DP - D, S), BF16)
    vT = _nt_dot(wqvT_v[D:D + DP, :], xn_v[...])
    rowv = jax.lax.broadcasted_iota(jnp.int32, (DP, S), 0)
    vT_v[...] = jnp.where((rowv & (HP - 1)) == DH, 1.0, vT).astype(BF16)

    row2 = jax.lax.broadcasted_iota(jnp.int32, (64, TQ), 0)

    def idx(i):
        return jax.lax.shift_right_logical(i, LQ), i & (NQ - 1)

    def get_q(i, hf):
        h, t = idx(i)
        g = jax.lax.shift_right_logical(h, 2)
        j = h & 3
        roff = pl.multiple_of(g * GW, 16)
        qoff = pl.multiple_of(t * TB + hf * TQ, TQ)
        q = qT_v[pl.ds(roff, 128), pl.ds(qoff, TQ)]
        q32 = pltpu.bitcast(q, jnp.uint32)
        keep = (row2 >= j * (DH // 2)) & (row2 < j * (DH // 2) + DH // 2)
        q32 = jnp.where(keep, q32, jnp.zeros_like(q32))
        return pltpu.bitcast(q32, BF16), pl.multiple_of(g * 128, 128)

    def qk_chunk(qm, goff, hf, c, s_w):
        k = k_v[pl.ds(c * TK, TK), pl.ds(goff, 128)]
        s = _dot(k, qm)
        s_w[pl.ds(c * TK, TK), pl.ds(hf * TQ, TQ)] = s
        return jnp.max(s.reshape(TK // 8, 8, TQ), axis=0)

    def step(i_cur, i_next, s_r, s_w):
        h, t = idx(i_cur)
        hoff = pl.multiple_of(h * HP, HP)
        for hf in range(NH):
            qm, goff = get_q(i_next, hf)
            m_cur = m_ref[:, pl.ds(hf * TQ, TQ)]
            m_next = None
            o = None
            for c in range(NC):
                mc = qk_chunk(qm, goff, hf, c, s_w)
                m_next = mc if m_next is None else jnp.maximum(m_next, mc)
                p = jnp.exp2(s_r[pl.ds(c * TK, TK), pl.ds(hf * TQ, TQ)] - m_cur).astype(BF16)
                vt = vT_v[pl.ds(hoff, HP), pl.ds(c * TK, TK)]
                oc = _dot(vt, p)
                o = oc if o is None else o + oc
            l = o[DH:DH + 1, :]
            o = o * (1.0 / l)
            oT_v[pl.ds(hoff, HP), pl.ds(pl.multiple_of(t * TB + hf * TQ, TQ), TQ)] = o.astype(BF16)
            m_ref[:, pl.ds(hf * TQ, TQ)] = jnp.max(m_next, axis=0, keepdims=True)

    for hf in range(NH):
        qm0, goff0 = get_q(0, hf)
        mm = None
        for c in range(NC):
            mc = qk_chunk(qm0, goff0, hf, c, sA)
            mm = mc if mm is None else jnp.maximum(mm, mc)
        m_ref[:, pl.ds(hf * TQ, TQ)] = jnp.max(mm, axis=0, keepdims=True)

    def body(i, carry):
        inext = jnp.minimum(i + 1, NBLK - 1)

        @pl.when((i & 1) == 0)
        def _():
            step(i, inext, sA, sB)

        @pl.when((i & 1) == 1)
        def _():
            step(i, inext, sB, sA)

        return carry

    jax.lax.fori_loop(0, NBLK, body, 0)

    cp_wo.wait()
    wof = wo_v[...].astype(F32)
    zpad = jnp.zeros((HP - DH, D), F32)
    wo_pad = jnp.concatenate(
        [blk for h in range(H) for blk in (wof[DH * h:DH * h + DH, :], zpad)], axis=0)
    woT_v[...] = wo_pad.T.astype(BF16)
    hT = xT_v[...] + _dot(woT_v[...], oT_v[...])
    hT_v[...] = hT
    mu2 = jnp.mean(hT, axis=0, keepdims=True)
    hc = hT - mu2
    var2 = jnp.mean(hc * hc, axis=0, keepdims=True)
    hnT_v[...] = (hc * jax.lax.rsqrt(var2 + EPS)).astype(BF16)

    cp_w1.wait()
    u = _dot(hnT_v[...], w1_v[...]) + b1_ref[...].astype(F32)
    g_v[...] = jax.nn.gelu(u, approximate=True).astype(BF16)
    cp_w2.wait()
    TO = 512
    out_cps = []
    for c in range(S // TO):
        y = _dot(g_v[...], w2_v[:, c * TO:(c + 1) * TO])
        h2 = hT_v[:, c * TO:(c + 1) * TO] + y + b2_ref[:, c * TO:(c + 1) * TO].astype(F32)
        out_v[c * TO:(c + 1) * TO, :] = h2.T.astype(BF16)
        cp = pltpu.make_async_copy(out_v.at[pl.ds(c * TO, TO), :],
                                   o_hbm.at[pl.ds(c * TO, TO), :], sems.at[5 + c])
        cp.start()
        out_cps.append(cp)
    for cp in out_cps:
        cp.wait()


@jax.jit
def pallas_sequential_preLN__mha_block__mixer_token_mlp__prompt_kernel(
    A_x: jax.Array,
    A_wqkv: jax.Array,
    A_wo: jax.Array,
    B_x: jax.Array,
    B_w1: jax.Array,
    B_b1: jax.Array,
    B_w2: jax.Array,
    B_b2: jax.Array,
):
    del B_x
    x = A_x.reshape(S, D)
    b1 = B_b1.reshape(1, F)
    b2 = B_b2.reshape(1, S)
    any_spec = pl.BlockSpec(memory_space=pl.ANY)
    vmem_spec = pl.BlockSpec(memory_space=pltpu.VMEM)
    scratch = [
        pltpu.VMEM((S, D), BF16),
        pltpu.VMEM((D, 3 * D), BF16),
        pltpu.VMEM((D, D), BF16),
        pltpu.VMEM((S, F), BF16),
        pltpu.VMEM((F, S), BF16),
        pltpu.VMEM((D + DP, D), BF16),
        pltpu.VMEM((D, DP), BF16),
        pltpu.VMEM((D, DP), BF16),
        pltpu.VMEM((S, D), BF16),
        pltpu.VMEM((D, S), F32),
        pltpu.VMEM((S, DP), BF16),
        pltpu.VMEM((DP, S), BF16),
        pltpu.VMEM((DP, S), BF16),
        pltpu.VMEM((DP, S), BF16),
        pltpu.VMEM((S, TB), F32),
        pltpu.VMEM((S, TB), F32),
        pltpu.VMEM((1, TB), F32),
        pltpu.VMEM((D, S), F32),
        pltpu.VMEM((D, S), BF16),
        pltpu.VMEM((D, F), BF16),
        pltpu.VMEM((S, D), BF16),
        pltpu.SemaphoreType.DMA((5 + S // 512,)),
    ]
    out = pl.pallas_call(
        _kernel,
        out_shape=jax.ShapeDtypeStruct((S, D), BF16),
        in_specs=[any_spec, any_spec, any_spec, any_spec, any_spec, vmem_spec, vmem_spec],
        out_specs=any_spec,
        scratch_shapes=scratch,
        compiler_params=pltpu.CompilerParams(vmem_limit_bytes=110 * 1024 * 1024),
    )(x, A_wqkv, A_wo, B_w1, B_w2, b1, b2)
    return out.reshape(1, S, D)
```

```python
import functools
import math

import jax
import jax.numpy as jnp
import jax.experimental.pallas as pl
import jax.experimental.pallas.tpu as pltpu

S = 2048
D = 448
H = 16
DH = 28
F = 1792
GW = 112
HP = 32
DP = H * HP
EPS = 1e-5
QSCALE = (DH ** -0.5) * math.log2(math.e)

TQ = 512
NH = 2
TB = TQ * NH
NQ = S // TB
LQ = NQ.bit_length() - 1
TK = 128
NC = S // TK
NBLK = H * NQ

F32 = jnp.float32
BF16 = jnp.bfloat16


def _nt_dot(a, b):
    return jax.lax.dot_general(a, b, (((1,), (1,)), ((), ())),
                               preferred_element_type=F32)


def _dot(a, b):
    return jnp.dot(a, b, preferred_element_type=F32)


def _kernel(x_hbm, wqkv_hbm, wo_hbm, w1_hbm, w2_hbm, b1_ref, b2_ref,
            o_hbm,
            x_v, wqkv_v, wo_v, w1_v, w2_v,
            wT_v, woT_v,
            xn_v, k_v, qT_v, vT_v, oT_v,
            sA, sB, m_ref, hT_v, hnT_v, g_v, out_v,
            sems):
    cp_wqkv = pltpu.make_async_copy(wqkv_hbm, wqkv_v, sems.at[0])
    cp_x = pltpu.make_async_copy(x_hbm, x_v, sems.at[1])
    cp_wo = pltpu.make_async_copy(wo_hbm, wo_v, sems.at[2])
    cp_w1 = pltpu.make_async_copy(w1_hbm, w1_v, sems.at[3])
    cp_w2 = pltpu.make_async_copy(w2_hbm, w2_v, sems.at[4])
    cp_wqkv.start()
    cp_x.start()
    cp_wo.start()
    cp_w1.start()
    cp_w2.start()

    cp_wqkv.wait()
    wT = wqkv_v[...].astype(F32).T
    wT_v[0:2 * D, :] = wT[0:2 * D, :].astype(BF16)
    wT_v[2 * D:2 * D + DP, :] = jnp.zeros((DP, D), BF16)
    for h in range(H):
        wT_v[2 * D + HP * h:2 * D + HP * h + DH, :] = (
            wT[2 * D + DH * h:2 * D + DH * h + DH, :].astype(BF16))

    cp_x.wait()
    xf = x_v[...].astype(F32)
    mu = jnp.mean(xf, axis=0, keepdims=True)
    xc = xf - mu
    var = jnp.mean(xc * xc, axis=0, keepdims=True)
    xn_v[...] = (xc * jax.lax.rsqrt(var + EPS)).astype(BF16)

    qT_v[0:D, :] = (_dot(wT_v[0:D, :], xn_v[...]) * QSCALE).astype(BF16)
    qT_v[D:DP, :] = jnp.zeros((DP - D, S), BF16)
    k_v[...] = jnp.zeros((S, DP), BF16)
    kT = _dot(wT_v[D:2 * D, :], xn_v[...])
    for g in range(4):
        k_v[:, 128 * g:128 * g + GW] = kT[GW * g:GW * g + GW, :].T.astype(BF16)
    vT = _dot(wT_v[2 * D:2 * D + DP, :], xn_v[...])
    rowv = jax.lax.broadcasted_iota(jnp.int32, (DP, S), 0)
    vT_v[...] = jnp.where((rowv & (HP - 1)) == DH, 1.0, vT).astype(BF16)

    row2 = jax.lax.broadcasted_iota(jnp.int32, (64, TQ), 0)

    def idx(i):
        return jax.lax.shift_right_logical(i, LQ), i & (NQ - 1)

    def get_q(i, hf):
        h, t = idx(i)
        g = jax.lax.shift_right_logical(h, 2)
        j = h & 3
        roff = pl.multiple_of(g * GW, 16)
        qoff = pl.multiple_of(t * TB + hf * TQ, TQ)
        q = qT_v[pl.ds(roff, 128), pl.ds(qoff, TQ)]
        q32 = pltpu.bitcast(q, jnp.uint32)
        keep = (row2 >= j * (DH // 2)) & (row2 < j * (DH // 2) + DH // 2)
        q32 = jnp.where(keep, q32, jnp.zeros_like(q32))
        return pltpu.bitcast(q32, BF16), pl.multiple_of(g * 128, 128)

    def qk_chunk(qm, goff, hf, c, s_w):
        k = k_v[pl.ds(c * TK, TK), pl.ds(goff, 128)]
        s = _dot(k, qm)
        s_w[pl.ds(c * TK, TK), pl.ds(hf * TQ, TQ)] = s
        return jnp.max(s.reshape(TK // 8, 8, TQ), axis=0)

    def step(i_cur, i_next, s_r, s_w):
        h, t = idx(i_cur)
        hoff = pl.multiple_of(h * HP, HP)
        for hf in range(NH):
            qm, goff = get_q(i_next, hf)
            m_cur = m_ref[:, pl.ds(hf * TQ, TQ)]
            m_next = None
            o = None
            for c in range(NC):
                mc = qk_chunk(qm, goff, hf, c, s_w)
                m_next = mc if m_next is None else jnp.maximum(m_next, mc)
                p = jnp.exp2(s_r[pl.ds(c * TK, TK), pl.ds(hf * TQ, TQ)] - m_cur).astype(BF16)
                vt = vT_v[pl.ds(hoff, HP), pl.ds(c * TK, TK)]
                oc = _dot(vt, p)
                o = oc if o is None else o + oc
            l = o[DH:DH + 1, :]
            o = o * (1.0 / l)
            oT_v[pl.ds(hoff, HP), pl.ds(pl.multiple_of(t * TB + hf * TQ, TQ), TQ)] = o.astype(BF16)
            m_ref[:, pl.ds(hf * TQ, TQ)] = jnp.max(m_next, axis=0, keepdims=True)

    for hf in range(NH):
        qm0, goff0 = get_q(0, hf)
        mm = None
        for c in range(NC):
            mc = qk_chunk(qm0, goff0, hf, c, sA)
            mm = mc if mm is None else jnp.maximum(mm, mc)
        m_ref[:, pl.ds(hf * TQ, TQ)] = jnp.max(mm, axis=0, keepdims=True)

    def body(i, carry):
        inext = jnp.minimum(i + 1, NBLK - 1)

        @pl.when((i & 1) == 0)
        def _():
            step(i, inext, sA, sB)

        @pl.when((i & 1) == 1)
        def _():
            step(i, inext, sB, sA)

        return carry

    jax.lax.fori_loop(0, NBLK, body, 0)

    cp_wo.wait()
    wof = wo_v[...].astype(F32)
    zpad = jnp.zeros((HP - DH, D), F32)
    wo_pad = jnp.concatenate(
        [blk for h in range(H) for blk in (wof[DH * h:DH * h + DH, :], zpad)], axis=0)
    woT_v[...] = wo_pad.T.astype(BF16)
    hT = x_v[...].astype(F32) + _dot(woT_v[...], oT_v[...])
    hT_v[...] = hT
    mu2 = jnp.mean(hT, axis=0, keepdims=True)
    hc = hT - mu2
    var2 = jnp.mean(hc * hc, axis=0, keepdims=True)
    hnT_v[...] = (hc * jax.lax.rsqrt(var2 + EPS)).astype(BF16)

    cp_w1.wait()
    u = _dot(hnT_v[...], w1_v[...]) + b1_ref[...].astype(F32).reshape(1, F)
    g_v[...] = jax.nn.gelu(u, approximate=True).astype(BF16)
    cp_w2.wait()
    TO = 512
    b2f = b2_ref[...].astype(F32).reshape(1, S)
    out_cps = []
    for c in range(S // TO):
        y = _dot(g_v[...], w2_v[:, c * TO:(c + 1) * TO])
        h2 = hT_v[:, c * TO:(c + 1) * TO] + y + b2f[:, c * TO:(c + 1) * TO]
        out_v[:, c * TO:(c + 1) * TO] = h2.astype(BF16)
        cp = pltpu.make_async_copy(out_v.at[:, pl.ds(c * TO, TO)],
                                   o_hbm.at[:, pl.ds(c * TO, TO)], sems.at[5 + c])
        cp.start()
        out_cps.append(cp)
    for cp in out_cps:
        cp.wait()


@jax.jit
def pallas_sequential_preLN__mha_block__mixer_token_mlp__prompt_kernel(
    A_x: jax.Array,
    A_wqkv: jax.Array,
    A_wo: jax.Array,
    B_x: jax.Array,
    B_w1: jax.Array,
    B_b1: jax.Array,
    B_w2: jax.Array,
    B_b2: jax.Array,
):
    del B_x
    x = A_x.reshape(S, D).T
    any_spec = pl.BlockSpec(memory_space=pltpu.MemorySpace.HBM)
    vmem_spec = pl.BlockSpec(memory_space=pltpu.VMEM)
    scratch = [
        pltpu.VMEM((D, S), BF16),
        pltpu.VMEM((D, 3 * D), BF16),
        pltpu.VMEM((D, D), BF16),
        pltpu.VMEM((S, F), BF16),
        pltpu.VMEM((F, S), BF16),
        pltpu.VMEM((2 * D + DP, D), BF16),
        pltpu.VMEM((D, DP), BF16),
        pltpu.VMEM((D, S), BF16),
        pltpu.VMEM((S, DP), BF16),
        pltpu.VMEM((DP, S), BF16),
        pltpu.VMEM((DP, S), BF16),
        pltpu.VMEM((DP, S), BF16),
        pltpu.VMEM((S, TB), F32),
        pltpu.VMEM((S, TB), F32),
        pltpu.VMEM((1, TB), F32),
        pltpu.VMEM((D, S), F32),
        pltpu.VMEM((D, S), BF16),
        pltpu.VMEM((D, F), BF16),
        pltpu.VMEM((D, S), BF16),
        pltpu.SemaphoreType.DMA((5 + S // 512,)),
    ]
    out = pl.pallas_call(
        _kernel,
        out_shape=jax.ShapeDtypeStruct((D, S), BF16),
        in_specs=[any_spec, any_spec, any_spec, any_spec, any_spec, vmem_spec, vmem_spec],
        out_specs=any_spec,
        scratch_shapes=scratch,
        compiler_params=pltpu.CompilerParams(vmem_limit_bytes=110 * 1024 * 1024),
    )(x, A_wqkv, A_wo, B_w1, B_w2, B_b1, B_b2)
    return out.T.reshape(1, S, D)
```

```python
import functools
import math

import jax
import jax.numpy as jnp
import jax.experimental.pallas as pl
import jax.experimental.pallas.tpu as pltpu

S = 2048
D = 448
H = 16
DH = 28
F = 1792
GW = 112
HP = 32
DP = H * HP
EPS = 1e-5
QSCALE = (DH ** -0.5) * math.log2(math.e)

TQ = 512
NH = S // TQ
TK = 128
NC = S // TK
TX = 512
NX = S // TX
TP = 128
NP = S // TP
FN = 128
OUT_CHUNKS = (512, 512, 512, 256, 128, 128)

F32 = jnp.float32
BF16 = jnp.bfloat16


def _dot(a, b):
    return jnp.dot(a, b, preferred_element_type=F32)


def _ln0(v):
    mu = jnp.mean(v, axis=0, keepdims=True)
    vc = v - mu
    var = jnp.mean(vc * vc, axis=0, keepdims=True)
    return vc * jax.lax.rsqrt(var + EPS)


def _kernel(x_hbm, wqkv_hbm, wo_hbm, w1_hbm, w2_hbm, b1_hbm, b2_hbm,
            o_hbm,
            x_v, wqkv_v, wo_v, w1_v, w2_v, b1_v, b2_v,
            wT_v, woT_v,
            xn_v, k_v, qT_v, vT_v, oT_v,
            sA, sB, m_ref, hT_v, hnT_v, g_v, out_v,
            sems):
    wcols = ((0, 512), (512, 384), (896, 448))
    cp_w = [pltpu.make_async_copy(wqkv_hbm.at[:, pl.ds(o, n)],
                                  wqkv_v.at[pl.ds(0, D), pl.ds(o, n)],
                                  sems.at[i]) for i, (o, n) in enumerate(wcols)]
    cp_x = [pltpu.make_async_copy(x_hbm.at[:, pl.ds(c * TX, TX)], x_v.at[:, pl.ds(c * TX, TX)],
                                  sems.at[3 + c]) for c in range(NX)]
    cp_wo = pltpu.make_async_copy(wo_hbm, wo_v, sems.at[3 + NX])
    cp_w1 = pltpu.make_async_copy(w1_hbm, w1_v, sems.at[4 + NX])
    cp_w2 = pltpu.make_async_copy(w2_hbm, w2_v, sems.at[5 + NX])
    cp_b1 = pltpu.make_async_copy(b1_hbm, b1_v, sems.at[6 + NX])
    cp_b2 = pltpu.make_async_copy(b2_hbm, b2_v, sems.at[7 + NX])
    cp_x[0].start()
    cp_w[0].start()
    cp_w[1].start()
    cp_w[2].start()
    for c in range(1, NX):
        cp_x[c].start()

    wqkv_v[D:DP, :] = jnp.zeros((DP - D, 3 * D), BF16)
    xn_v[D:DP, :] = jnp.zeros((DP - D, S), BF16)
    qT_v[D:DP, :] = jnp.zeros((DP - D, S), BF16)
    wT_v[2 * D:2 * D + DP, :] = jnp.zeros((DP, DP), BF16)

    rowv = jax.lax.broadcasted_iota(jnp.int32, (DP, TP), 0)
    is_one = (rowv & (HP - 1)) == DH

    def tsl(t):
        return slice(t * TP, (t + 1) * TP)

    def ln1(t):
        xn_v[0:D, tsl(t)] = _ln0(x_v[:, tsl(t)].astype(F32)).astype(BF16)

    def q_p(t):
        qT_v[0:D, tsl(t)] = (_dot(wT_v[0:D, :], xn_v[:, tsl(t)]) * QSCALE).astype(BF16)

    def k_p(t):
        kT = _dot(wT_v[D:2 * D, :], xn_v[:, tsl(t)])
        zr = jnp.zeros((128 - GW, TP), F32)
        for g in range(4):
            kg = jnp.concatenate([kT[GW * g:GW * g + GW, :], zr], axis=0)
            k_v[tsl(t), 128 * g:128 * g + 128] = kg.T.astype(BF16)

    def v_p(t):
        vT = _dot(wT_v[2 * D:2 * D + DP, :], xn_v[:, tsl(t)])
        vT_v[:, tsl(t)] = jnp.where(is_one, 1.0, vT).astype(BF16)

    def wt_block(j):
        wT_v[128 * j:128 * j + 128, :] = (
            wqkv_v[:, 128 * j:128 * j + 128].astype(F32).T.astype(BF16))

    def wv_prep():
        wvT = wqkv_v[:, 2 * D:3 * D].astype(F32).T
        for h in range(H):
            wT_v[2 * D + HP * h:2 * D + HP * h + DH, :] = (
                wvT[DH * h:DH * h + DH, :].astype(BF16))

    cp_x[0].wait()
    cp_w[0].wait()
    for j in range(4):
        wt_block(j)
    ln1(0)
    for t in range(4):
        if t < 3:
            ln1(t + 1)
        q_p(t)
    cp_w[1].wait()
    cp_w[2].wait()
    cp_x[1].wait()
    ln1(4)
    wt_block(4)
    ln1(5)
    q_p(4)
    wt_block(5)
    ln1(6)
    q_p(5)
    wt_block(6)
    ln1(7)
    q_p(6)
    wv_prep()
    q_p(7)
    for t in range(4):
        k_p(t)
        v_p(t)
    for c in range(2, NX):
        cp_x[c].wait()
    cp_wo.start()
    cp_b1.start()
    cp_b2.start()
    cp_w1.start()
    cp_w2.start()
    ln1(8)
    for t in range(4, 8):
        k_p(t)
        ln1(t + 5)
        v_p(t)
    for t in range(8, NP):
        q_p(t)
        k_p(t)
        if t + 5 < NP:
            ln1(t + 5)
        v_p(t)

    row2 = jax.lax.broadcasted_iota(jnp.int32, (64, TQ), 0)

    def get_q(h, hf):
        g = jax.lax.shift_right_logical(h, 2)
        j = h & 3
        roff = pl.multiple_of(g * GW, 16)
        q = qT_v[pl.ds(roff, 128), pl.ds(hf * TQ, TQ)]
        q32 = pltpu.bitcast(q, jnp.uint32)
        keep = (row2 >= j * (DH // 2)) & (row2 < j * (DH // 2) + DH // 2)
        q32 = jnp.where(keep, q32, jnp.zeros_like(q32))
        return pltpu.bitcast(q32, BF16), pl.multiple_of(g * 128, 128)

    def qk_chunk(qm, goff, hf, c, s_w):
        k = k_v[pl.ds(c * TK, TK), pl.ds(goff, 128)]
        s = _dot(k, qm)
        s_w[pl.ds(c * TK, TK), pl.ds(hf * TQ, TQ)] = s
        return jnp.max(s.reshape(TK // 8, 8, TQ), axis=0)

    def step(h_cur, h_next, s_r, s_w, extra=None):
        for hf in range(NH):
            if h_next is not None:
                qm, goff = get_q(h_next, hf)
            if h_cur is not None:
                hoff = pl.multiple_of(h_cur * HP, HP)
                m_cur = m_ref[:, pl.ds(hf * TQ, TQ)]
            m_next = None
            o = None
            for c in range(NC):
                if h_next is not None:
                    mc = qk_chunk(qm, goff, hf, c, s_w)
                    m_next = mc if m_next is None else jnp.maximum(m_next, mc)
                if h_cur is not None:
                    p = jnp.exp2(s_r[pl.ds(c * TK, TK), pl.ds(hf * TQ, TQ)] - m_cur).astype(BF16)
                    vt = vT_v[pl.ds(hoff, HP), pl.ds(c * TK, TK)]
                    oc = _dot(vt, p)
                    o = oc if o is None else o + oc
                if extra is not None:
                    extra(hf, c)
            if h_cur is not None:
                l = o[DH:DH + 1, :]
                o = o * (1.0 / l)
                oT_v[pl.ds(hoff, HP), pl.ds(hf * TQ, TQ)] = o.astype(BF16)
            if h_next is not None:
                m_ref[:, pl.ds(hf * TQ, TQ)] = jnp.max(m_next, axis=0, keepdims=True)

    cp_wo.wait()

    def wo_prep(hf, c):
        if hf == 0 and c == 2:
            wof = wo_v[...].astype(F32)
            zpad = jnp.zeros((HP - DH, D), F32)
            wo_pad = jnp.concatenate(
                [blk for h in range(H) for blk in (wof[DH * h:DH * h + DH, :], zpad)], axis=0)
            woT_v[...] = wo_pad.T.astype(BF16)

    step(None, 0, None, sA, extra=wo_prep)

    def body(h, carry):
        @pl.when((h & 1) == 0)
        def _():
            step(h, h + 1, sA, sB)

        @pl.when((h & 1) == 1)
        def _():
            step(h, h + 1, sB, sA)

        return carry

    jax.lax.fori_loop(0, H - 1, body, 0)

    cp_w1.wait()
    cp_w2.wait()
    cp_b1.wait()
    cp_b2.wait()

    KP = 384

    def wo_rest_ln(t):
        hT = hT_v[:, tsl(t)] + _dot(woT_v[:, KP:DP], oT_v[KP:DP, tsl(t)])
        hT_v[:, tsl(t)] = hT
        hnT_v[:, tsl(t)] = _ln0(hT).astype(BF16)

    def wo_part(hf, c):
        if c % 4 == 3:
            t = hf * 4 + c // 4
            hT_v[:, tsl(t)] = x_v[:, tsl(t)].astype(F32) + _dot(woT_v[:, 0:KP], oT_v[0:KP, tsl(t)])
        if hf in (1, 2) and c % 8 == 5:
            wo_rest_ln((hf - 1) * 2 + c // 8)

    step(H - 1, None, sB, None, extra=wo_part)

    NF = F // FN
    u = [None] * NF
    for c in range(NH):
        cs = slice(c * TQ, (c + 1) * TQ)
        for n in range(NF):
            d = _dot(hnT_v[:, cs], w1_v[cs, n * FN:(n + 1) * FN])
            u[n] = d if u[n] is None else u[n] + d
            if c + 1 < NH and n % 3 == 1 and n // 3 < 4:
                wo_rest_ln((c + 1) * 4 + n // 3)
            if c + 1 == NH:
                ns = slice(n * FN, (n + 1) * FN)
                un = u[n] + b1_v[ns].astype(F32).reshape(1, FN)
                g_v[:, ns] = jax.nn.gelu(un, approximate=True).astype(BF16)
    b2f = b2_v[...].astype(F32).reshape(1, S)
    out_cps = []
    t0 = 0
    for i, n in enumerate(OUT_CHUNKS):
        cs = slice(t0, t0 + n)
        y = _dot(g_v[...], w2_v[:, cs])
        h2 = hT_v[:, cs] + y + b2f[:, cs]
        out_v[:, cs] = h2.astype(BF16)
        cp = pltpu.make_async_copy(out_v.at[:, pl.ds(t0, n)],
                                   o_hbm.at[:, pl.ds(t0, n)], sems.at[8 + NX + i])
        cp.start()
        out_cps.append(cp)
        t0 += n
    for cp in out_cps:
        cp.wait()


@jax.jit
def pallas_sequential_preLN__mha_block__mixer_token_mlp__prompt_kernel(
    A_x: jax.Array,
    A_wqkv: jax.Array,
    A_wo: jax.Array,
    B_x: jax.Array,
    B_w1: jax.Array,
    B_b1: jax.Array,
    B_w2: jax.Array,
    B_b2: jax.Array,
):
    del B_x
    x = A_x.reshape(S, D).T
    hbm_spec = pl.BlockSpec(memory_space=pltpu.MemorySpace.HBM)
    scratch = [
        pltpu.VMEM((D, S), BF16),
        pltpu.VMEM((DP, 3 * D), BF16),
        pltpu.VMEM((D, D), BF16),
        pltpu.VMEM((S, F), BF16),
        pltpu.VMEM((F, S), BF16),
        pltpu.VMEM((F,), BF16),
        pltpu.VMEM((S,), BF16),
        pltpu.VMEM((2 * D + DP, DP), BF16),
        pltpu.VMEM((D, DP), BF16),
        pltpu.VMEM((DP, S), BF16),
        pltpu.VMEM((S, DP), BF16),
        pltpu.VMEM((DP, S), BF16),
        pltpu.VMEM((DP, S), BF16),
        pltpu.VMEM((DP, S), BF16),
        pltpu.VMEM((S, S), F32),
        pltpu.VMEM((S, S), F32),
        pltpu.VMEM((1, S), F32),
        pltpu.VMEM((D, S), F32),
        pltpu.VMEM((D, S), BF16),
        pltpu.VMEM((D, F), BF16),
        pltpu.VMEM((D, S), BF16),
        pltpu.SemaphoreType.DMA((8 + NX + len(OUT_CHUNKS),)),
    ]
    out = pl.pallas_call(
        _kernel,
        out_shape=jax.ShapeDtypeStruct((D, S), BF16),
        in_specs=[hbm_spec] * 7,
        out_specs=hbm_spec,
        scratch_shapes=scratch,
        compiler_params=pltpu.CompilerParams(vmem_limit_bytes=120 * 1024 * 1024),
    )(x, A_wqkv, A_wo, B_w1, B_w2, B_b1, B_b2)
    return out.T.reshape(1, S, D)
```

```python
import math

import jax
import jax.numpy as jnp
import jax.experimental.pallas as pl
import jax.experimental.pallas.tpu as pltpu

S = 2048
D = 448
H = 16
DH = 28
F = 1792
GW = 112
HP = 32
DP = H * HP
EPS = 1e-5
QSCALE = (DH ** -0.5) * math.log2(math.e)

TQ = 512
NH = S // TQ
TK = 128
NC = S // TK
TX = 512
NX = S // TX
TP = 128
NP = S // TP
KP = 384
ELN = 2
KCH = 256
FN = 256
OUT_CHUNKS = (512, 512, 512, 256, 128, 128)

F32 = jnp.float32
BF16 = jnp.bfloat16


def _dot(a, b):
    return jnp.dot(a, b, preferred_element_type=F32)


def _ln0(v):
    mu = jnp.mean(v, axis=0, keepdims=True)
    vc = v - mu
    var = jnp.mean(vc * vc, axis=0, keepdims=True)
    return vc * jax.lax.rsqrt(var + EPS)


def _tsl(t):
    return slice(t * TP, (t + 1) * TP)


def _kernel(x_hbm, wqkv_hbm, wo_hbm, w1_hbm, w2_hbm, b1_hbm, b2_hbm,
            o_hbm,
            x_v, wqkv_v, wo_v, w1_v, w2_v, b1_v, b2_v,
            wT_v, woT_v,
            xn_v, k_v, qT_v, vT_v, oT_v,
            sA, sB, m_ref, hT_v, hnT_v, g_v, out_v,
            sems):
    wcols = ((0, 512), (512, 384), (896, 448))
    cp_w = [pltpu.make_async_copy(wqkv_hbm.at[:, pl.ds(o, n)],
                                  wqkv_v.at[pl.ds(0, D), pl.ds(o, n)],
                                  sems.at[i]) for i, (o, n) in enumerate(wcols)]
    cp_x = [pltpu.make_async_copy(x_hbm.at[:, pl.ds(c * TX, TX)],
                                  x_v.at[:, pl.ds(c * TX, TX)],
                                  sems.at[3 + c]) for c in range(NX)]
    cp_wo = pltpu.make_async_copy(wo_hbm, wo_v, sems.at[3 + NX])
    cp_w1 = pltpu.make_async_copy(w1_hbm, w1_v, sems.at[4 + NX])
    cp_w2 = pltpu.make_async_copy(w2_hbm, w2_v, sems.at[5 + NX])
    cp_b1 = pltpu.make_async_copy(b1_hbm, b1_v, sems.at[6 + NX])
    cp_b2 = pltpu.make_async_copy(b2_hbm, b2_v, sems.at[7 + NX])
    cp_x[0].start()
    cp_w[0].start()
    cp_w[1].start()
    cp_w[2].start()
    for c in range(1, NX):
        cp_x[c].start()

    wqkv_v[D:DP, :] = jnp.zeros((DP - D, 3 * D), BF16)
    xn_v[D:DP, :] = jnp.zeros((DP - D, S), BF16)
    qT_v[D:DP, :] = jnp.zeros((DP - D, S), BF16)

    tail4 = (jax.lax.broadcasted_iota(jnp.int32, (HP - DH, TP), 0) == 0).astype(F32)

    def ln1(t):
        xn_v[0:D, _tsl(t)] = _ln0(x_v[:, _tsl(t)].astype(F32)).astype(BF16)

    def q_p(t):
        qT_v[0:D, _tsl(t)] = (_dot(wT_v[0:D, :], xn_v[:, _tsl(t)]) * QSCALE).astype(BF16)

    def k_p(t):
        kT = _dot(wT_v[D:2 * D, :], xn_v[:, _tsl(t)])
        zr = jnp.zeros((128 - GW, TP), F32)
        for g in range(4):
            kg = jnp.concatenate([kT[GW * g:GW * g + GW, :], zr], axis=0)
            k_v[_tsl(t), 128 * g:128 * g + 128] = kg.T.astype(BF16)

    def v_p(t):
        vT = _dot(wT_v[2 * D:3 * D, :], xn_v[:, _tsl(t)])
        blks = []
        for h in range(H):
            blks.append(vT[DH * h:DH * h + DH, :])
            blks.append(tail4)
        vT_v[:, _tsl(t)] = jnp.concatenate(blks, axis=0).astype(BF16)

    def wt_block(j):
        wT_v[128 * j:128 * j + 128, :] = (
            wqkv_v[:, 128 * j:128 * j + 128].astype(F32).T.astype(BF16))

    def wv_prep():
        wT_v[2 * D:3 * D, :] = wqkv_v[:, 2 * D:3 * D].astype(F32).T.astype(BF16)

    cp_x[0].wait()
    cp_w[0].wait()
    for j in range(4):
        wt_block(j)
    ln1(0)
    for t in range(4):
        if t < 3:
            ln1(t + 1)
        q_p(t)

    cp_w[1].wait()
    cp_w[2].wait()
    cp_x[1].wait()
    ln1(4)
    wt_block(4)
    ln1(5)
    q_p(4)
    wt_block(5)
    ln1(6)
    q_p(5)
    wt_block(6)
    ln1(7)
    q_p(6)
    wv_prep()
    q_p(7)
    for t in range(4):
        k_p(t)
        v_p(t)

    for c in range(2, NX):
        cp_x[c].wait()
    cp_wo.start()
    cp_b1.start()
    cp_b2.start()
    cp_w1.start()
    cp_w2.start()
    ln1(8)
    for t in range(4, 8):
        k_p(t)
        ln1(t + 5)
        v_p(t)
    for t in range(8, NP):
        q_p(t)
        k_p(t)
        if t + 5 < NP:
            ln1(t + 5)
        v_p(t)

    row2 = jax.lax.broadcasted_iota(jnp.int32, (64, TQ), 0)

    def get_q(h, hf):
        g = jax.lax.shift_right_logical(h, 2)
        j = h & 3
        roff = pl.multiple_of(g * GW, 16)
        q = qT_v[pl.ds(roff, 128), pl.ds(hf * TQ, TQ)]
        q32 = pltpu.bitcast(q, jnp.uint32)
        keep = (row2 >= j * (DH // 2)) & (row2 < j * (DH // 2) + DH // 2)
        q32 = jnp.where(keep, q32, jnp.zeros_like(q32))
        return pltpu.bitcast(q32, BF16), pl.multiple_of(g * 128, 128)

    def step(h_cur, h_next, s_r, s_w, extra=None):
        for hf in range(NH):
            qs = pl.ds(hf * TQ, TQ)
            if h_next is not None:
                qm, goff = get_q(h_next, hf)
            if h_cur is not None:
                hoff = pl.multiple_of(h_cur * HP, HP)
                m_cur = m_ref[:, qs]
            m_next = None
            o = None
            for c in range(NC):
                ks = pl.ds(c * TK, TK)
                if h_cur is not None:
                    p = jnp.exp2(s_r[ks, qs] - m_cur).astype(BF16)
                    oc = _dot(vT_v[pl.ds(hoff, HP), ks], p)
                    o = oc if o is None else o + oc
                if h_next is not None:
                    s = _dot(k_v[ks, pl.ds(goff, 128)], qm)
                    s_w[ks, qs] = s
                    mc = jnp.max(s.reshape(TK // 8, 8, TQ), axis=0)
                    m_next = mc if m_next is None else jnp.maximum(m_next, mc)
                if extra is not None:
                    extra(hf, c)
            if h_cur is not None:
                l = o[DH:DH + 1, :]
                o = o * (1.0 / l)
                oT_v[pl.ds(hoff, HP), qs] = o.astype(BF16)
            if h_next is not None:
                m_ref[:, qs] = jnp.max(m_next, axis=0, keepdims=True)

    cp_wo.wait()

    def wo_prep(hf, c):
        if hf == 0 and c == 2:
            wof = wo_v[...].astype(F32)
            zpad = jnp.zeros((HP - DH, D), F32)
            wo_pad = jnp.concatenate(
                [blk for h in range(H) for blk in (wof[DH * h:DH * h + DH, :], zpad)], axis=0)
            woT_v[...] = wo_pad.T.astype(BF16)

    step(None, 0, None, sA, extra=wo_prep)

    def body(h, carry):
        @pl.when((h & 1) == 0)
        def _():
            step(h, h + 1, sA, sB)

        @pl.when((h & 1) == 1)
        def _():
            step(h, h + 1, sB, sA)

        return carry

    jax.lax.fori_loop(0, H - 1, body, 0)

    cp_w1.wait()
    cp_w2.wait()
    cp_b1.wait()
    cp_b2.wait()

    def wo_rest_ln(t):
        hT = hT_v[:, _tsl(t)] + _dot(woT_v[:, KP:DP], oT_v[KP:DP, _tsl(t)])
        hT_v[:, _tsl(t)] = hT
        hnT_v[:, _tsl(t)] = _ln0(hT).astype(BF16)

    def wo_part(hf, c):
        if c % 4 == 3:
            t = hf * 4 + c // 4
            hT_v[:, _tsl(t)] = (x_v[:, _tsl(t)].astype(F32)
                                + _dot(woT_v[:, 0:KP], oT_v[0:KP, _tsl(t)]))
        if 1 <= hf <= ELN and c == 9:
            wo_rest_ln(hf - 1)

    step(H - 1, None, sB, None, extra=wo_part)

    NF = F // FN
    KC = KCH // TP
    NK = S // KCH
    u = [None] * NF
    done = ELN
    for c in range(NK):
        while done < (c + 1) * KC:
            wo_rest_ln(done)
            done += 1
        cs = slice(c * KCH, (c + 1) * KCH)
        nxt = list(range(done, min(NP, (c + 2) * KC)))
        sched = {}
        for i, t in enumerate(nxt):
            sched.setdefault(((i + 1) * NF) // (len(nxt) + 1), []).append(t)
        for n in range(NF):
            ns = slice(n * FN, (n + 1) * FN)
            d = _dot(hnT_v[:, cs], w1_v[cs, ns])
            u[n] = d if u[n] is None else u[n] + d
            for t in sched.get(n, ()):
                wo_rest_ln(t)
                done += 1
            if c + 1 == NK:
                un = u[n] + b1_v[ns].astype(F32).reshape(1, FN)
                g_v[:, ns] = jax.nn.gelu(un, approximate=True).astype(BF16)

    b2f = b2_v[...].astype(F32).reshape(1, S)
    out_cps = []
    t0 = 0
    for i, n in enumerate(OUT_CHUNKS):
        cs = slice(t0, t0 + n)
        y = _dot(g_v[...], w2_v[:, cs])
        h2 = hT_v[:, cs] + y + b2f[:, cs]
        out_v[:, cs] = h2.astype(BF16)
        cp = pltpu.make_async_copy(out_v.at[:, pl.ds(t0, n)],
                                   o_hbm.at[:, pl.ds(t0, n)], sems.at[8 + NX + i])
        cp.start()
        out_cps.append(cp)
        t0 += n
    for cp in out_cps:
        cp.wait()


@jax.jit
def pallas_sequential_preLN__mha_block__mixer_token_mlp__prompt_kernel(
    A_x: jax.Array,
    A_wqkv: jax.Array,
    A_wo: jax.Array,
    B_x: jax.Array,
    B_w1: jax.Array,
    B_b1: jax.Array,
    B_w2: jax.Array,
    B_b2: jax.Array,
):
    del B_x
    x = A_x.reshape(S, D).T
    hbm_spec = pl.BlockSpec(memory_space=pltpu.MemorySpace.HBM)
    scratch = [
        pltpu.VMEM((D, S), BF16),
        pltpu.VMEM((DP, 3 * D), BF16),
        pltpu.VMEM((D, D), BF16),
        pltpu.VMEM((S, F), BF16),
        pltpu.VMEM((F, S), BF16),
        pltpu.VMEM((F,), BF16),
        pltpu.VMEM((S,), BF16),
        pltpu.VMEM((3 * D, DP), BF16),
        pltpu.VMEM((D, DP), BF16),
        pltpu.VMEM((DP, S), BF16),
        pltpu.VMEM((S, DP), BF16),
        pltpu.VMEM((DP, S), BF16),
        pltpu.VMEM((DP, S), BF16),
        pltpu.VMEM((DP, S), BF16),
        pltpu.VMEM((S, S), F32),
        pltpu.VMEM((S, S), F32),
        pltpu.VMEM((1, S), F32),
        pltpu.VMEM((D, S), F32),
        pltpu.VMEM((D, S), BF16),
        pltpu.VMEM((D, F), BF16),
        pltpu.VMEM((D, S), BF16),
        pltpu.SemaphoreType.DMA((8 + NX + len(OUT_CHUNKS),)),
    ]
    out = pl.pallas_call(
        _kernel,
        out_shape=jax.ShapeDtypeStruct((D, S), BF16),
        in_specs=[hbm_spec] * 7,
        out_specs=hbm_spec,
        scratch_shapes=scratch,
        compiler_params=pltpu.CompilerParams(vmem_limit_bytes=120 * 1024 * 1024),
    )(x, A_wqkv, A_wo, B_w1, B_w2, B_b1, B_b2)
    return out.T.reshape(1, S, D)
```

```python
import math

import jax
import jax.numpy as jnp
import jax.experimental.pallas as pl
import jax.experimental.pallas.tpu as pltpu

S = 2048
D = 448
H = 16
DH = 28
F = 1792
GW = 112
HP = 32
DP = H * HP
EPS = 1e-5
QSCALE = (DH ** -0.5) * math.log2(math.e)

TQ = 512
NH = S // TQ
TK = 128
NC = S // TK
TX = 512
NX = S // TX
TP = 128
NP = S // TP
KP = 384
ELN = 2
KCH = 256
FN = 256
OUT_CHUNKS = (512, 512, 512, 256, 128, 128)

F32 = jnp.float32
BF16 = jnp.bfloat16


def _dot(a, b):
    return jnp.dot(a, b, preferred_element_type=F32)


def _ln0(v):
    mu = jnp.mean(v, axis=0, keepdims=True)
    vc = v - mu
    var = jnp.mean(vc * vc, axis=0, keepdims=True)
    return vc * jax.lax.rsqrt(var + EPS)


def _tsl(t):
    return slice(t * TP, (t + 1) * TP)


def _kernel(x_hbm, wqkv_hbm, wo_hbm, w1_hbm, w2_hbm, b1_hbm, b2_hbm,
            o_hbm,
            x_v, wqkv_v, wo_v, w1_v, w2_v, b1_v, b2_v,
            wT_v, woT_v,
            xn_v, k_v, qT_v, vT_v, oT_v,
            sA, sB, m_ref, hT_v, hnT_v, g_v, out_v,
            sems):
    wcols = ((0, 256), (256, 256), (512, 384), (896, 448))
    xcols = ((0, 256), (256, 256), (512, 512), (1024, 1024))
    cp_w = [pltpu.make_async_copy(wqkv_hbm.at[:, pl.ds(o, n)],
                                  wqkv_v.at[pl.ds(0, D), pl.ds(o, n)],
                                  sems.at[i]) for i, (o, n) in enumerate(wcols)]
    cp_x = [pltpu.make_async_copy(x_hbm.at[:, pl.ds(o, n)],
                                  x_v.at[:, pl.ds(o, n)],
                                  sems.at[4 + i]) for i, (o, n) in enumerate(xcols)]
    cp_wo = pltpu.make_async_copy(wo_hbm, wo_v, sems.at[8])
    cp_w1 = pltpu.make_async_copy(w1_hbm, w1_v, sems.at[9])
    cp_w2 = pltpu.make_async_copy(w2_hbm, w2_v, sems.at[10])
    cp_b1 = pltpu.make_async_copy(b1_hbm, b1_v, sems.at[11])
    cp_b2 = pltpu.make_async_copy(b2_hbm, b2_v, sems.at[12])
    cp_x[0].start()
    cp_w[0].start()
    cp_w[1].start()
    cp_x[1].start()
    cp_x[2].start()
    cp_w[2].start()
    cp_w[3].start()
    cp_x[3].start()

    wqkv_v[D:DP, :] = jnp.zeros((DP - D, 3 * D), BF16)
    xn_v[D:DP, :] = jnp.zeros((DP - D, S), BF16)
    qT_v[D:DP, :] = jnp.zeros((DP - D, S), BF16)

    tail4 = (jax.lax.broadcasted_iota(jnp.int32, (HP - DH, TP), 0) == 0).astype(F32)

    def ln1(t):
        xn_v[0:D, _tsl(t)] = _ln0(x_v[:, _tsl(t)].astype(F32)).astype(BF16)

    def q_p(t, r0=0, r1=D):
        qT_v[r0:r1, _tsl(t)] = (_dot(wT_v[r0:r1, :], xn_v[:, _tsl(t)]) * QSCALE).astype(BF16)

    def k_p(t):
        kT = _dot(wT_v[D:2 * D, :], xn_v[:, _tsl(t)])
        zr = jnp.zeros((128 - GW, TP), F32)
        for g in range(4):
            kg = jnp.concatenate([kT[GW * g:GW * g + GW, :], zr], axis=0)
            k_v[_tsl(t), 128 * g:128 * g + 128] = kg.T.astype(BF16)

    def v_p(t):
        vT = _dot(wT_v[2 * D:3 * D, :], xn_v[:, _tsl(t)])
        blks = []
        for h in range(H):
            blks.append(vT[DH * h:DH * h + DH, :])
            blks.append(tail4)
        vT_v[:, _tsl(t)] = jnp.concatenate(blks, axis=0).astype(BF16)

    def wt_block(j):
        wT_v[128 * j:128 * j + 128, :] = (
            wqkv_v[:, 128 * j:128 * j + 128].astype(F32).T.astype(BF16))

    def wv_prep():
        wT_v[2 * D:3 * D, :] = wqkv_v[:, 2 * D:3 * D].astype(F32).T.astype(BF16)

    cp_x[0].wait()
    cp_w[0].wait()
    wt_block(0)
    ln1(0)
    wt_block(1)
    ln1(1)
    q_p(0, 0, 256)
    q_p(1, 0, 256)

    cp_w[1].wait()
    cp_x[1].wait()
    wt_block(2)
    wt_block(3)
    ln1(2)
    q_p(0, 256, D)
    ln1(3)
    q_p(1, 256, D)
    q_p(2)
    q_p(3)

    cp_x[2].wait()
    ln1(4)
    ln1(5)
    q_p(4)
    ln1(6)
    q_p(5)

    cp_w[2].wait()
    cp_w[3].wait()
    wt_block(4)
    ln1(7)
    q_p(6)
    wt_block(5)
    wt_block(6)
    q_p(7)
    wv_prep()
    for t in range(4):
        k_p(t)
        v_p(t)

    cp_x[3].wait()
    cp_wo.start()
    cp_b1.start()
    cp_b2.start()
    cp_w1.start()
    cp_w2.start()
    ln1(8)
    for t in range(4, 8):
        k_p(t)
        ln1(t + 5)
        v_p(t)
    for t in range(8, NP):
        q_p(t)
        k_p(t)
        if t + 5 < NP:
            ln1(t + 5)
        v_p(t)

    row2 = jax.lax.broadcasted_iota(jnp.int32, (64, TQ), 0)

    def get_q(h, hf):
        g = jax.lax.shift_right_logical(h, 2)
        j = h & 3
        roff = pl.multiple_of(g * GW, 16)
        q = qT_v[pl.ds(roff, 128), pl.ds(hf * TQ, TQ)]
        q32 = pltpu.bitcast(q, jnp.uint32)
        keep = (row2 >= j * (DH // 2)) & (row2 < j * (DH // 2) + DH // 2)
        q32 = jnp.where(keep, q32, jnp.zeros_like(q32))
        return pltpu.bitcast(q32, BF16), pl.multiple_of(g * 128, 128)

    def step(h_cur, h_next, s_r, s_w, extra=None):
        for hf in range(NH):
            qs = pl.ds(hf * TQ, TQ)
            if h_next is not None:
                qm, goff = get_q(h_next, hf)
            if h_cur is not None:
                hoff = pl.multiple_of(h_cur * HP, HP)
                m_cur = m_ref[:, qs]
            m_next = None
            o = None
            for c in range(NC):
                ks = pl.ds(c * TK, TK)
                if h_cur is not None:
                    p = jnp.exp2(s_r[ks, qs] - m_cur).astype(BF16)
                    oc = _dot(vT_v[pl.ds(hoff, HP), ks], p)
                    o = oc if o is None else o + oc
                if h_next is not None:
                    s = _dot(k_v[ks, pl.ds(goff, 128)], qm)
                    s_w[ks, qs] = s
                    mc = jnp.max(s.reshape(TK // 8, 8, TQ), axis=0)
                    m_next = mc if m_next is None else jnp.maximum(m_next, mc)
                if extra is not None:
                    extra(hf, c)
            if h_cur is not None:
                l = o[DH:DH + 1, :]
                o = o * (1.0 / l)
                oT_v[pl.ds(hoff, HP), qs] = o.astype(BF16)
            if h_next is not None:
                m_ref[:, qs] = jnp.max(m_next, axis=0, keepdims=True)

    cp_wo.wait()

    def wo_prep(hf, c):
        if hf == 0 and c == 2:
            wof = wo_v[...].astype(F32)
            zpad = jnp.zeros((HP - DH, D), F32)
            wo_pad = jnp.concatenate(
                [blk for h in range(H) for blk in (wof[DH * h:DH * h + DH, :], zpad)], axis=0)
            woT_v[...] = wo_pad.T.astype(BF16)

    step(None, 0, None, sA, extra=wo_prep)

    def body(h, carry):
        @pl.when((h & 1) == 0)
        def _():
            step(h, h + 1, sA, sB)

        @pl.when((h & 1) == 1)
        def _():
            step(h, h + 1, sB, sA)

        return carry

    jax.lax.fori_loop(0, H - 1, body, 0)

    cp_w1.wait()
    cp_w2.wait()
    cp_b1.wait()
    cp_b2.wait()

    def wo_rest_ln(t):
        hT = hT_v[:, _tsl(t)] + _dot(woT_v[:, KP:DP], oT_v[KP:DP, _tsl(t)])
        hT_v[:, _tsl(t)] = hT
        hnT_v[:, _tsl(t)] = _ln0(hT).astype(BF16)

    def wo_part(hf, c):
        if c % 4 == 3:
            t = hf * 4 + c // 4
            hT_v[:, _tsl(t)] = (x_v[:, _tsl(t)].astype(F32)
                                + _dot(woT_v[:, 0:KP], oT_v[0:KP, _tsl(t)]))
        if 1 <= hf <= ELN and c == 9:
            wo_rest_ln(hf - 1)

    step(H - 1, None, sB, None, extra=wo_part)

    NF = F // FN
    KC = KCH // TP
    NK = S // KCH
    u = [None] * NF
    done = ELN
    for c in range(NK):
        while done < (c + 1) * KC:
            wo_rest_ln(done)
            done += 1
        cs = slice(c * KCH, (c + 1) * KCH)
        nxt = list(range(done, min(NP, (c + 2) * KC)))
        sched = {}
        for i, t in enumerate(nxt):
            sched.setdefault(((i + 1) * NF) // (len(nxt) + 1), []).append(t)
        for n in range(NF):
            ns = slice(n * FN, (n + 1) * FN)
            d = _dot(hnT_v[:, cs], w1_v[cs, ns])
            u[n] = d if u[n] is None else u[n] + d
            for t in sched.get(n, ()):
                wo_rest_ln(t)
                done += 1
            if c + 1 == NK:
                un = u[n] + b1_v[ns].astype(F32).reshape(1, FN)
                g_v[:, ns] = jax.nn.gelu(un, approximate=True).astype(BF16)

    b2f = b2_v[...].astype(F32).reshape(1, S)
    out_cps = []
    t0 = 0
    for i, n in enumerate(OUT_CHUNKS):
        cs = slice(t0, t0 + n)
        y = _dot(g_v[...], w2_v[:, cs])
        h2 = hT_v[:, cs] + y + b2f[:, cs]
        out_v[:, cs] = h2.astype(BF16)
        cp = pltpu.make_async_copy(out_v.at[:, pl.ds(t0, n)],
                                   o_hbm.at[:, pl.ds(t0, n)], sems.at[13 + i])
        cp.start()
        out_cps.append(cp)
        t0 += n
    for cp in out_cps:
        cp.wait()


@jax.jit
def pallas_sequential_preLN__mha_block__mixer_token_mlp__prompt_kernel(
    A_x: jax.Array,
    A_wqkv: jax.Array,
    A_wo: jax.Array,
    B_x: jax.Array,
    B_w1: jax.Array,
    B_b1: jax.Array,
    B_w2: jax.Array,
    B_b2: jax.Array,
):
    del B_x
    x = A_x.reshape(S, D).T
    hbm_spec = pl.BlockSpec(memory_space=pltpu.MemorySpace.HBM)
    scratch = [
        pltpu.VMEM((D, S), BF16),
        pltpu.VMEM((DP, 3 * D), BF16),
        pltpu.VMEM((D, D), BF16),
        pltpu.VMEM((S, F), BF16),
        pltpu.VMEM((F, S), BF16),
        pltpu.VMEM((F,), BF16),
        pltpu.VMEM((S,), BF16),
        pltpu.VMEM((3 * D, DP), BF16),
        pltpu.VMEM((D, DP), BF16),
        pltpu.VMEM((DP, S), BF16),
        pltpu.VMEM((S, DP), BF16),
        pltpu.VMEM((DP, S), BF16),
        pltpu.VMEM((DP, S), BF16),
        pltpu.VMEM((DP, S), BF16),
        pltpu.VMEM((S, S), F32),
        pltpu.VMEM((S, S), F32),
        pltpu.VMEM((1, S), F32),
        pltpu.VMEM((D, S), F32),
        pltpu.VMEM((D, S), BF16),
        pltpu.VMEM((D, F), BF16),
        pltpu.VMEM((D, S), BF16),
        pltpu.SemaphoreType.DMA((13 + len(OUT_CHUNKS),)),
    ]
    out = pl.pallas_call(
        _kernel,
        out_shape=jax.ShapeDtypeStruct((D, S), BF16),
        in_specs=[hbm_spec] * 7,
        out_specs=hbm_spec,
        scratch_shapes=scratch,
        compiler_params=pltpu.CompilerParams(vmem_limit_bytes=120 * 1024 * 1024),
    )(x, A_wqkv, A_wo, B_w1, B_w2, B_b1, B_b2)
    return out.T.reshape(1, S, D)
```

```python
import math

import jax
import jax.numpy as jnp
import jax.experimental.pallas as pl
import jax.experimental.pallas.tpu as pltpu

S = 2048
D = 448
H = 16
DH = 28
F = 1792
GW = 112
HP = 32
DP = H * HP
EPS = 1e-5
QSCALE = (DH ** -0.5) * math.log2(math.e)

TQ = 512
NH = S // TQ
TK = 128
NC = S // TK
TX = 512
NX = S // TX
TP = 128
NP = S // TP
KP = 384
KCH = 256
FN = 256
OUT_CHUNKS = (512, 512, 512, 256, 128, 128)

F32 = jnp.float32
BF16 = jnp.bfloat16


def _dot(a, b):
    return jnp.dot(a, b, preferred_element_type=F32)


def _ln0(v):
    mu = jnp.mean(v, axis=0, keepdims=True)
    vc = v - mu
    var = jnp.mean(vc * vc, axis=0, keepdims=True)
    return vc * jax.lax.rsqrt(var + EPS)


def _tsl(t):
    return slice(t * TP, (t + 1) * TP)


def _kernel(x_hbm, wqkv_hbm, wo_hbm, w1_hbm, w2_hbm, b1_hbm, b2_hbm,
            o_hbm,
            x_v, wqkv_v, wo_v, w1_v, w2_v, b1_v, b2_v,
            wT_v, woT_v,
            xn_v, k_v, qT_v, vT_v, oT_v,
            sA, sB, m_ref, hT_v, hnT_v, g_v, out_v,
            sems):
    wcols = ((0, 256), (256, 256), (512, 384), (896, 448))
    xcols = ((0, 256), (256, 256), (512, 512), (1024, 1024))
    cp_w = [pltpu.make_async_copy(wqkv_hbm.at[:, pl.ds(o, n)],
                                  wqkv_v.at[pl.ds(0, D), pl.ds(o, n)],
                                  sems.at[i]) for i, (o, n) in enumerate(wcols)]
    cp_x = [pltpu.make_async_copy(x_hbm.at[:, pl.ds(o, n)],
                                  x_v.at[:, pl.ds(o, n)],
                                  sems.at[4 + i]) for i, (o, n) in enumerate(xcols)]
    cp_wo = pltpu.make_async_copy(wo_hbm, wo_v, sems.at[8])
    cp_w1 = pltpu.make_async_copy(w1_hbm, w1_v, sems.at[9])
    cp_w2 = pltpu.make_async_copy(w2_hbm, w2_v, sems.at[10])
    cp_b1 = pltpu.make_async_copy(b1_hbm, b1_v, sems.at[11])
    cp_b2 = pltpu.make_async_copy(b2_hbm, b2_v, sems.at[12])
    cp_x[0].start()
    cp_w[0].start()
    cp_w[1].start()
    cp_x[1].start()
    cp_x[2].start()
    cp_w[2].start()
    cp_w[3].start()
    cp_x[3].start()

    wqkv_v[D:DP, :] = jnp.zeros((DP - D, 3 * D), BF16)
    xn_v[D:DP, :] = jnp.zeros((DP - D, S), BF16)
    qT_v[D:DP, :] = jnp.zeros((DP - D, S), BF16)

    tail4 = (jax.lax.broadcasted_iota(jnp.int32, (HP - DH, TP), 0) == 0).astype(F32)

    def ln1(t):
        xn_v[0:D, _tsl(t)] = _ln0(x_v[:, _tsl(t)].astype(F32)).astype(BF16)

    def q_p(t, r0=0, r1=D):
        qT_v[r0:r1, _tsl(t)] = (_dot(wT_v[r0:r1, :], xn_v[:, _tsl(t)]) * QSCALE).astype(BF16)

    def k_p(t):
        kT = _dot(wT_v[D:2 * D, :], xn_v[:, _tsl(t)])
        zr = jnp.zeros((128 - GW, TP), F32)
        for g in range(4):
            kg = jnp.concatenate([kT[GW * g:GW * g + GW, :], zr], axis=0)
            k_v[_tsl(t), 128 * g:128 * g + 128] = kg.T.astype(BF16)

    def v_p(t):
        vT = _dot(wT_v[2 * D:3 * D, :], xn_v[:, _tsl(t)])
        blks = []
        for h in range(H):
            blks.append(vT[DH * h:DH * h + DH, :])
            blks.append(tail4)
        vT_v[:, _tsl(t)] = jnp.concatenate(blks, axis=0).astype(BF16)

    def wt_block(j):
        wT_v[128 * j:128 * j + 128, :] = (
            wqkv_v[:, 128 * j:128 * j + 128].astype(F32).T.astype(BF16))

    def wv_prep():
        wT_v[2 * D:3 * D, :] = wqkv_v[:, 2 * D:3 * D].astype(F32).T.astype(BF16)

    cp_x[0].wait()
    cp_w[0].wait()
    wt_block(0)
    ln1(0)
    wt_block(1)
    ln1(1)
    q_p(0, 0, 256)
    q_p(1, 0, 256)

    cp_w[1].wait()
    cp_x[1].wait()
    wt_block(2)
    wt_block(3)
    ln1(2)
    q_p(0, 256, D)
    ln1(3)
    q_p(1, 256, D)
    q_p(2)
    q_p(3)

    cp_x[2].wait()
    ln1(4)
    ln1(5)
    q_p(4)
    ln1(6)
    q_p(5)

    cp_w[2].wait()
    cp_w[3].wait()
    wt_block(4)
    ln1(7)
    q_p(6)
    wt_block(5)
    wt_block(6)
    q_p(7)
    wv_prep()
    for t in range(4):
        k_p(t)
        v_p(t)

    cp_x[3].wait()
    cp_wo.start()
    cp_b1.start()
    cp_b2.start()
    cp_w1.start()
    cp_w2.start()
    ln1(8)
    for t in range(4, 8):
        k_p(t)
        ln1(t + 5)
        v_p(t)
    for t in range(8, NP):
        q_p(t)
        k_p(t)
        if t + 5 < NP:
            ln1(t + 5)
        v_p(t)

    row2 = jax.lax.broadcasted_iota(jnp.int32, (64, TQ), 0)

    def get_q(h, hf):
        g = jax.lax.shift_right_logical(h, 2)
        j = h & 3
        roff = pl.multiple_of(g * GW, 16)
        q = qT_v[pl.ds(roff, 128), pl.ds(hf * TQ, TQ)]
        q32 = pltpu.bitcast(q, jnp.uint32)
        keep = (row2 >= j * (DH // 2)) & (row2 < j * (DH // 2) + DH // 2)
        q32 = jnp.where(keep, q32, jnp.zeros_like(q32))
        return pltpu.bitcast(q32, BF16), pl.multiple_of(g * 128, 128)

    def step(h_cur, h_next, s_r, s_w, extra=None):
        for hf in range(NH):
            qs = pl.ds(hf * TQ, TQ)
            if h_next is not None:
                qm, goff = get_q(h_next, hf)
            if h_cur is not None:
                hoff = pl.multiple_of(h_cur * HP, HP)
                m_cur = m_ref[:, qs]
            m_next = None
            o = None
            for c in range(NC):
                ks = pl.ds(c * TK, TK)
                if h_cur is not None:
                    p = jnp.exp2(s_r[ks, qs] - m_cur).astype(BF16)
                    oc = _dot(vT_v[pl.ds(hoff, HP), ks], p)
                    o = oc if o is None else o + oc
                if h_next is not None:
                    s = _dot(k_v[ks, pl.ds(goff, 128)], qm)
                    s_w[ks, qs] = s
                    mc = jnp.max(s.reshape(TK // 8, 8, TQ), axis=0)
                    m_next = mc if m_next is None else jnp.maximum(m_next, mc)
                if extra is not None:
                    extra(hf, c)
            if h_cur is not None:
                l = o[DH:DH + 1, :]
                o = o * (1.0 / l)
                oT_v[pl.ds(hoff, HP), qs] = o.astype(BF16)
            if h_next is not None:
                m_ref[:, qs] = jnp.max(m_next, axis=0, keepdims=True)

    cp_wo.wait()

    def wo_prep(hf, c):
        if hf == 0 and c == 2:
            wof = wo_v[...].astype(F32)
            zpad = jnp.zeros((HP - DH, D), F32)
            wo_pad = jnp.concatenate(
                [blk for h in range(H) for blk in (wof[DH * h:DH * h + DH, :], zpad)], axis=0)
            woT_v[...] = wo_pad.T.astype(BF16)

    step(None, 0, None, sA, extra=wo_prep)

    def body(h, carry):
        @pl.when((h & 1) == 0)
        def _():
            step(h, h + 1, sA, sB)

        @pl.when((h & 1) == 1)
        def _():
            step(h, h + 1, sB, sA)

        return carry

    jax.lax.fori_loop(0, H - 1, body, 0)

    cp_w1.wait()
    cp_w2.wait()
    cp_b1.wait()
    cp_b2.wait()

    def wo_rest_ln(t):
        hT = hT_v[:, _tsl(t)] + _dot(woT_v[:, KP:DP], oT_v[KP:DP, _tsl(t)])
        hT_v[:, _tsl(t)] = hT
        hnT_v[:, _tsl(t)] = _ln0(hT).astype(BF16)

    NF = F // FN
    KC = KCH // TP
    NK = S // KCH
    u = [None] * NF

    def mix1(c, n):
        cs = slice(c * KCH, (c + 1) * KCH)
        ns = slice(n * FN, (n + 1) * FN)
        d = _dot(hnT_v[:, cs], w1_v[cs, ns])
        u[n] = d if u[n] is None else u[n] + d
        if c + 1 == NK:
            un = u[n] + b1_v[ns].astype(F32).reshape(1, FN)
            g_v[:, ns] = jax.nn.gelu(un, approximate=True).astype(BF16)

    def wo_part(hf, c):
        if c % 4 == 3:
            t = hf * 4 + c // 4
            hT_v[:, _tsl(t)] = (x_v[:, _tsl(t)].astype(F32)
                                + _dot(woT_v[:, 0:KP], oT_v[0:KP, _tsl(t)]))
        if hf in (1, 2) and c % 8 == 5:
            wo_rest_ln((hf - 1) * 2 + c // 8)

    step(H - 1, None, sB, None, extra=wo_part)

    done = 4
    for c in range(NK):
        while done < (c + 1) * KC:
            wo_rest_ln(done)
            done += 1
        nxt = list(range(done, min(NP, (c + 2) * KC)))
        sched = {}
        for i, t in enumerate(nxt):
            sched.setdefault(((i + 1) * NF) // (len(nxt) + 1), []).append(t)
        for n in range(NF):
            mix1(c, n)
            for t in sched.get(n, ()):
                wo_rest_ln(t)
                done += 1

    b2f = b2_v[...].astype(F32).reshape(1, S)
    out_cps = []
    t0 = 0
    for i, n in enumerate(OUT_CHUNKS):
        cs = slice(t0, t0 + n)
        y = _dot(g_v[...], w2_v[:, cs])
        h2 = hT_v[:, cs] + y + b2f[:, cs]
        out_v[:, cs] = h2.astype(BF16)
        cp = pltpu.make_async_copy(out_v.at[:, pl.ds(t0, n)],
                                   o_hbm.at[:, pl.ds(t0, n)], sems.at[13 + i])
        cp.start()
        out_cps.append(cp)
        t0 += n
    for cp in out_cps:
        cp.wait()


@jax.jit
def pallas_sequential_preLN__mha_block__mixer_token_mlp__prompt_kernel(
    A_x: jax.Array,
    A_wqkv: jax.Array,
    A_wo: jax.Array,
    B_x: jax.Array,
    B_w1: jax.Array,
    B_b1: jax.Array,
    B_w2: jax.Array,
    B_b2: jax.Array,
):
    del B_x
    x = A_x.reshape(S, D).T
    hbm_spec = pl.BlockSpec(memory_space=pltpu.MemorySpace.HBM)
    scratch = [
        pltpu.VMEM((D, S), BF16),
        pltpu.VMEM((DP, 3 * D), BF16),
        pltpu.VMEM((D, D), BF16),
        pltpu.VMEM((S, F), BF16),
        pltpu.VMEM((F, S), BF16),
        pltpu.VMEM((F,), BF16),
        pltpu.VMEM((S,), BF16),
        pltpu.VMEM((3 * D, DP), BF16),
        pltpu.VMEM((D, DP), BF16),
        pltpu.VMEM((DP, S), BF16),
        pltpu.VMEM((S, DP), BF16),
        pltpu.VMEM((DP, S), BF16),
        pltpu.VMEM((DP, S), BF16),
        pltpu.VMEM((DP, S), BF16),
        pltpu.VMEM((S, S), F32),
        pltpu.VMEM((S, S), F32),
        pltpu.VMEM((1, S), F32),
        pltpu.VMEM((D, S), F32),
        pltpu.VMEM((D, S), BF16),
        pltpu.VMEM((D, F), BF16),
        pltpu.VMEM((D, S), BF16),
        pltpu.SemaphoreType.DMA((13 + len(OUT_CHUNKS),)),
    ]
    out = pl.pallas_call(
        _kernel,
        out_shape=jax.ShapeDtypeStruct((D, S), BF16),
        in_specs=[hbm_spec] * 7,
        out_specs=hbm_spec,
        scratch_shapes=scratch,
        compiler_params=pltpu.CompilerParams(vmem_limit_bytes=120 * 1024 * 1024),
    )(x, A_wqkv, A_wo, B_w1, B_w2, B_b1, B_b2)
    return out.T.reshape(1, S, D)
```
